```python
import os as _os
_os.environ.setdefault('JAX_PLATFORMS', 'cpu')
import jax
import jax.numpy as jnp

def _softmax(x, axis=-1):
    return jax.nn.softmax(x, axis=axis)

def _gelu(x):
    return jax.nn.gelu(x, approximate=True)

def _silu(x):
    return jax.nn.silu(x)

def _sigmoid(x):
    return jax.nn.sigmoid(x)

def _layernorm(x, axis=-1, eps=1e-05):
    m = jnp.mean(x, axis=axis, keepdims=True)
    v = jnp.var(x, axis=axis, keepdims=True)
    return (x - m) / jnp.sqrt(v + eps)

def _scatter_add(tgt, idx, src, axis=0):
    return tgt.at[idx].add(src)

def _segment_sum(src, seg, n):
    return jax.ops.segment_sum(src, seg, n)

class _Rng:

    def __init__(self, key):
        self._k = key

    def _next(self):
        self._k, sub = jax.random.split(self._k)
        return sub

    def normal(self, shape):
        return jax.random.normal(self._next(), shape, dtype=jnp.bfloat16)

    def randint(self, lo, hi, shape):
        return jax.random.randint(self._next(), shape, lo, hi, dtype=jnp.int32)

    def uniform(self, shape, lo=0.0, hi=1.0):
        return jax.random.uniform(self._next(), shape, jnp.bfloat16, lo, hi)

    def permutation(self, n):
        return jax.random.permutation(self._next(), n)
kernel_name = 'adaLN_cond__sliding_local_dilated__dense_activation_relu__prompt'

def setup_inputs():
    _rng = _Rng(jax.random.key(int.from_bytes(__import__("os").urandom(4), "little")))
    _w = lambda a: (lambda t: t.astype(jnp.bfloat16) if jnp.issubdtype(t.dtype, jnp.floating) else t)(jnp.asarray(a))

    def _A_setup():
        B, S, D = (1, 2048, 576)
        return {'x': _w((lambda *s: _rng.normal(s) * 0.05)(B, S, D)), 'wqkv': _w((lambda *s: _rng.normal(s) * 0.05)(D, 3 * D)), 'wo': _w((lambda *s: _rng.normal(s) * 0.05)(D, D))}
    _A_in = _A_setup()

    def _B_setup():
        B, S, D, Dff = (1, 2048, 576, 4608)
        return {'x': _w((lambda *s: _rng.normal(s) * 0.05)(B, S, D)), 'w1': _w((lambda *s: _rng.normal(s) * 0.05)(D, Dff)), 'w2': _w((lambda *s: _rng.normal(s) * 0.05)(Dff, D))}
    _B_in = _B_setup()
    return {'A_x': _A_in['x'], 'A_wqkv': _A_in['wqkv'], 'A_wo': _A_in['wo'], 'B_x': _B_in['x'], 'B_w1': _B_in['w1'], 'B_w2': _B_in['w2'], 'c': _w((lambda *s: _rng.normal(s) * 0.05)(1, 576) * 8.0), 'w_mod': _w((lambda *s: _rng.normal(s) * 0.05)(576, 6 * 576) * 576 ** (-0.5) * 8.0)}

def reference(A_x, A_wqkv, A_wo, B_x, B_w1, B_w2, c, w_mod):

    def _A_ref(x, wqkv, wo):
        B, S, D = x.shape
        H = 32
        Dh = D // H
        W, dil = (8, 2)
        qkv = (lambda x, *d: x.transpose(*d))((x @ wqkv).reshape(B, S, 3, H, Dh), 2, 0, 3, 1, 4)
        q, k, v = (qkv[0], qkv[1], qkv[2])
        scale = Dh ** (-0.5)
        pos = jnp.arange(S)
        off = jnp.arange(W) * dil
        idx = pos[:, None] - off[None, :]
        mask = idx >= 0
        idx_c = jnp.where(mask, idx, 0).reshape(-1)
        kg = k[:, :, idx_c, :].reshape(B, H, S, W, Dh)
        vg = v[:, :, idx_c, :].reshape(B, H, S, W, Dh)
        logits = jnp.einsum('bhsd,bhswd->bhsw', q, kg) * scale
        logits = jnp.where(mask[None, None, :, :], logits, -1000000000.0)
        attn = _softmax(logits, axis=-1)
        o = jnp.einsum('bhsw,bhswd->bhsd', attn, vg)
        return (lambda x, *d: x.transpose(*d))(o, 0, 2, 1, 3).reshape(B, S, D) @ wo

    def _B_ref(x, w1, w2):
        h = jnp.einsum('bsd,df->bsf', x, w1)
        zero = jnp.zeros_like(h)
        h = jnp.maximum(h, zero)
        return jnp.einsum('bsf,fd->bsd', h, w2)
    x = A_x
    mod = (_silu(c) @ w_mod).reshape(c.shape[0], 6, 1, -1)
    sa, ca, ga, sb, cb, gb = (mod[:, 0].copy(), mod[:, 1].copy(), mod[:, 2].copy(), mod[:, 3].copy(), mod[:, 4].copy(), mod[:, 5].copy())
    h = _layernorm(x, axis=-1) * (1 + ca) + sa
    x = x + ga * _A_ref(h, A_wqkv, A_wo)
    h = _layernorm(x, axis=-1) * (1 + cb) + sb
    x = x + gb * _B_ref(h, B_w1, B_w2)
    return x
```

```python
import functools

import jax
import jax.numpy as jnp
import jax.experimental.pallas as pl
import jax.experimental.pallas.tpu as pltpu

H = 32
W = 8
DIL = 2
HALO = 16
EPS = 1e-5
LANES = 128
NT = (((1,), (1,)), ((), ()))
TN = (((0,), (0,)), ((), ()))


def _kernel(x_ref, c_ref, wqkv_hbm, wo_hbm, w1_hbm, w2t_hbm, wmod_hbm, o_ref,
            wq_raw, wo_raw, wq_s, woT_s, w1_s, w2t_s, wmod_s, modT_s, kbuf, vbuf, sems,
            *, T, D, DP, DFF, FC):
    i = pl.program_id(0)
    Dh = D // H
    f32 = jnp.float32
    bf16 = jnp.bfloat16

    @pl.when(i == 0)
    def _init():
        cps = [
            pltpu.make_async_copy(wmod_hbm, wmod_s, sems.at[0]),
            pltpu.make_async_copy(wqkv_hbm, wq_raw, sems.at[1]),
            pltpu.make_async_copy(wo_hbm, wo_raw, sems.at[2]),
            pltpu.make_async_copy(w1_hbm, w1_s, sems.at[3]),
            pltpu.make_async_copy(w2t_hbm, w2t_s, sems.at[4]),
        ]
        cps[1].start()
        cps[2].start()
        cps[0].start()
        kbuf[0:HALO, :] = jnp.zeros((HALO, DP), f32)
        vbuf[0:HALO, :] = jnp.zeros((HALO, DP), f32)
        cps[1].wait()
        cps[3].start()
        cps[4].start()
        for j in range(3):
            start = (j * D) // LANES * LANES
            width = j * D + D - start
            r = jax.lax.broadcasted_iota(jnp.int32, (width, DP), 0) - (j * D - start)
            col_ = jax.lax.broadcasted_iota(jnp.int32, (width, DP), 1)
            tgt = (r % Dh) * H + r // Dh
            Pj = jnp.where((r >= 0) & (col_ == tgt), 1.0, 0.0).astype(bf16)
            wq_s[:, j * DP:(j + 1) * DP] = jnp.dot(
                wq_raw[:, start:start + width], Pj, preferred_element_type=f32).astype(bf16)
        cps[2].wait()
        rr = jax.lax.broadcasted_iota(jnp.int32, (D, DP), 0)
        cc = jax.lax.broadcasted_iota(jnp.int32, (D, DP), 1)
        P = jnp.where(cc == (rr % Dh) * H + rr // Dh, 1.0, 0.0).astype(bf16)
        woT_s[...] = jax.lax.dot_general(
            wo_raw[...], P, TN, preferred_element_type=f32).astype(bf16)
        c = c_ref[...].astype(f32)
        sc = (c * jax.nn.sigmoid(c)).astype(bf16)
        scb = jnp.broadcast_to(sc, (16, D))
        cps[0].wait()
        modb = jnp.dot(scb, wmod_s[...], preferred_element_type=f32)
        modT_s[...] = jnp.broadcast_to(modb.T[:, 0:1], (6 * D, LANES))

    reps = T // LANES

    def col(j):
        m = modT_s[j * D:(j + 1) * D, :]
        return jnp.concatenate([m] * reps, axis=1) if reps > 1 else m

    x = x_ref[...].astype(f32)
    m = jnp.mean(x, axis=0, keepdims=True)
    xc = x - m
    v = jnp.mean(xc * xc, axis=0, keepdims=True)
    hT = xc * jax.lax.rsqrt(v + EPS) * (1.0 + col(1)) + col(0)
    h = hT.T.astype(bf16)

    qkv = jnp.dot(h, wq_s[...], preferred_element_type=f32)
    q = qkv[:, 0:DP]
    kbuf[HALO:HALO + T, :] = qkv[:, DP:2 * DP]
    vbuf[HALO:HALO + T, :] = qkv[:, 2 * DP:3 * DP]

    scale = Dh ** (-0.5)
    row = jax.lax.broadcasted_iota(jnp.int32, (T, LANES), 0) + i * T
    logits = []
    for w in range(W):
        kw = kbuf[pl.ds(HALO - DIL * w, T), :]
        p = q * kw
        s = p[:, 0:LANES]
        for j in range(1, DP // LANES):
            s = s + p[:, j * LANES:(j + 1) * LANES]
        s = s + pltpu.roll(s, 64, axis=1)
        s = s + pltpu.roll(s, 32, axis=1)
        s = s * scale
        if w > 0:
            s = jnp.where(row >= DIL * w, s, -1000000000.0)
        logits.append(s)
    mx = logits[0]
    for w in range(1, W):
        mx = jnp.maximum(mx, logits[w])
    es = [jnp.exp(l - mx) for l in logits]
    den = es[0]
    for w in range(1, W):
        den = den + es[w]
    inv = 1.0 / den
    ps = [e * inv for e in es]
    ocols = []
    for j in range(DP // LANES):
        acc = None
        for w in range(W):
            t = ps[w] * vbuf[pl.ds(HALO - DIL * w, T), j * LANES:(j + 1) * LANES]
            acc = t if acc is None else acc + t
        ocols.append(acc.astype(bf16))
    o = jnp.concatenate(ocols, axis=1)

    kbuf[0:HALO, :] = kbuf[T:T + HALO, :]
    vbuf[0:HALO, :] = vbuf[T:T + HALO, :]

    att = jax.lax.dot_general(woT_s[...], o, NT, preferred_element_type=f32)
    x1 = x + col(2) * att

    m2 = jnp.mean(x1, axis=0, keepdims=True)
    xc2 = x1 - m2
    v2 = jnp.mean(xc2 * xc2, axis=0, keepdims=True)
    h2T = (xc2 * jax.lax.rsqrt(v2 + EPS) * (1.0 + col(4)) + col(3))
    h2 = h2T.T.astype(bf16)

    @pl.when(i == 0)
    def _wait_ffn():
        pltpu.make_async_copy(w1_hbm, w1_s, sems.at[3]).wait()
        pltpu.make_async_copy(w2t_hbm, w2t_s, sems.at[4]).wait()

    acc = None
    for cidx in range(DFF // FC):
        a = jnp.dot(h2, w1_s[:, cidx * FC:(cidx + 1) * FC], preferred_element_type=f32)
        a = jnp.maximum(a, 0.0).astype(bf16)
        t = jax.lax.dot_general(w2t_s[:, cidx * FC:(cidx + 1) * FC], a, NT,
                                preferred_element_type=f32)
        acc = t if acc is None else acc + t
    o_ref[...] = (x1 + col(5) * acc).astype(o_ref.dtype)


@jax.jit
def pallas_adaLN_cond__sliding_local_dilated__dense_activation_relu__prompt_kernel(
    A_x: jax.Array,
    A_wqkv: jax.Array,
    A_wo: jax.Array,
    B_x: jax.Array,
    B_w1: jax.Array,
    B_w2: jax.Array,
    c: jax.Array,
    w_mod: jax.Array,
):
    B, S, D = A_x.shape
    assert B == 1
    DFF = B_w1.shape[1]
    Dh = D // H
    DP = ((Dh + 3) // 4) * 4 * H
    assert DP % LANES == 0
    T = 256
    FC = 512
    xT = jnp.swapaxes(A_x, 1, 2).reshape(D, S)
    w2T = B_w2.T
    f32 = jnp.float32
    bf16 = jnp.bfloat16
    kern = functools.partial(_kernel, T=T, D=D, DP=DP, DFF=DFF, FC=FC)
    any_spec = pl.BlockSpec(memory_space=pltpu.MemorySpace.HBM)
    outT = pl.pallas_call(
        kern,
        grid=(S // T,),
        in_specs=[
            pl.BlockSpec((D, T), lambda i: (0, i)),
            pl.BlockSpec((1, D), lambda i: (0, 0)),
            any_spec, any_spec, any_spec, any_spec, any_spec,
        ],
        out_specs=pl.BlockSpec((D, T), lambda i: (0, i)),
        out_shape=jax.ShapeDtypeStruct((D, S), A_x.dtype),
        scratch_shapes=[
            pltpu.VMEM((D, 3 * D), bf16),
            pltpu.VMEM((D, D), bf16),
            pltpu.VMEM((D, 3 * DP), bf16),
            pltpu.VMEM((D, DP), bf16),
            pltpu.VMEM((D, DFF), bf16),
            pltpu.VMEM((D, DFF), bf16),
            pltpu.VMEM((D, 6 * D), bf16),
            pltpu.VMEM((6 * D, LANES), f32),
            pltpu.VMEM((T + HALO, DP), f32),
            pltpu.VMEM((T + HALO, DP), f32),
            pltpu.SemaphoreType.DMA((5,)),
        ],
        compiler_params=pltpu.CompilerParams(
            dimension_semantics=("arbitrary",),
            vmem_limit_bytes=100 * 1024 * 1024,
        ),
    )(xT, c, A_wqkv, A_wo, B_w1, w2T, w_mod)
    return jnp.swapaxes(outT.reshape(B, D, S), 1, 2)
```

```python
import functools

import jax
import jax.numpy as jnp
import jax.experimental.pallas as pl
import jax.experimental.pallas.tpu as pltpu

H = 32
W = 8
DIL = 2
HALO = 16
EPS = 1e-5
LANES = 128
NT = (((1,), (1,)), ((), ()))
TN = (((0,), (0,)), ((), ()))


def _kernel(x_ref, c_ref, wqkv_hbm, wo_hbm, w1_hbm, w2t_hbm, wmod_hbm, o_ref,
            wq_raw, wo_raw, wq_s, woT_s, w1_s, w2t_s, wmod_s, modT_s, kbuf, vbuf, sems,
            *, T, D, DP, DFF, FC):
    i = pl.program_id(0)
    Dh = D // H
    f32 = jnp.float32
    bf16 = jnp.bfloat16

    @pl.when(i == 0)
    def _init():
        cps = [
            pltpu.make_async_copy(wmod_hbm, wmod_s, sems.at[0]),
            pltpu.make_async_copy(wqkv_hbm, wq_raw, sems.at[1]),
            pltpu.make_async_copy(wo_hbm, wo_raw, sems.at[2]),
            pltpu.make_async_copy(w1_hbm, w1_s, sems.at[3]),
            pltpu.make_async_copy(w2t_hbm, w2t_s, sems.at[4]),
        ]
        cps[1].start()
        cps[2].start()
        cps[0].start()
        kbuf[0:HALO, :] = jnp.zeros((HALO, DP), f32)
        vbuf[0:HALO, :] = jnp.zeros((HALO, DP), f32)
        def perm(width, shift):
            r = jax.lax.broadcasted_iota(jnp.int32, (width, DP), 0) - shift
            col_ = jax.lax.broadcasted_iota(jnp.int32, (width, DP), 1)
            tgt = (r % Dh) * H + r // Dh
            return jnp.where((r >= 0) & (col_ == tgt), 1.0, 0.0).astype(bf16)

        shifts = [(j * D) % LANES for j in range(3)]
        perms = {sh: perm(D + sh, sh) for sh in sorted(set(shifts + [0]))}
        cps[1].wait()
        cps[3].start()
        cps[4].start()
        for j in range(3):
            start = j * D - shifts[j]
            wq_s[:, j * DP:(j + 1) * DP] = jnp.dot(
                wq_raw[:, start:start + D + shifts[j]], perms[shifts[j]],
                preferred_element_type=f32).astype(bf16)
        cps[2].wait()
        woT_s[...] = jax.lax.dot_general(
            wo_raw[...], perms[0], TN, preferred_element_type=f32).astype(bf16)
        c = c_ref[...].astype(f32)
        sc = (c * jax.nn.sigmoid(c)).astype(bf16)
        scb = jnp.broadcast_to(sc, (16, D))
        cps[0].wait()
        modb = jnp.dot(scb, wmod_s[...], preferred_element_type=f32)
        modT_s[...] = jnp.broadcast_to(modb.T[:, 0:1], (6 * D, LANES))

    reps = T // LANES

    def col(j):
        m = modT_s[j * D:(j + 1) * D, :]
        return jnp.concatenate([m] * reps, axis=1) if reps > 1 else m

    x = x_ref[...].astype(f32)
    m = jnp.mean(x, axis=0, keepdims=True)
    xc = x - m
    v = jnp.mean(xc * xc, axis=0, keepdims=True)
    hT = xc * jax.lax.rsqrt(v + EPS) * (1.0 + col(1)) + col(0)
    h = hT.T.astype(bf16)

    qkv = jnp.dot(h, wq_s[...], preferred_element_type=f32)
    q = qkv[:, 0:DP]
    kbuf[HALO:HALO + T, :] = qkv[:, DP:2 * DP]
    vbuf[HALO:HALO + T, :] = qkv[:, 2 * DP:3 * DP]

    scale = Dh ** (-0.5)
    row = jax.lax.broadcasted_iota(jnp.int32, (T, LANES), 0) + i * T
    def windows(buf):
        base = {r: buf[pl.ds(r, T + HALO - (8 if r else 0)), :] for r in range(0, 8, DIL)}
        out = []
        for w in range(W):
            off = HALO - DIL * w
            out.append(base[off % 8][off - off % 8:off - off % 8 + T, :])
        return out

    kws = windows(kbuf)
    logits = []
    for w in range(W):
        kw = kws[w]
        p = q * kw
        s = p[:, 0:LANES]
        for j in range(1, DP // LANES):
            s = s + p[:, j * LANES:(j + 1) * LANES]
        s = s + pltpu.roll(s, 64, axis=1)
        s = s + pltpu.roll(s, 32, axis=1)
        s = s * scale
        if w > 0:
            s = jnp.where(row >= DIL * w, s, -1000000000.0)
        logits.append(s)
    mx = logits[0]
    for w in range(1, W):
        mx = jnp.maximum(mx, logits[w])
    es = [jnp.exp(l - mx) for l in logits]
    den = es[0]
    for w in range(1, W):
        den = den + es[w]
    inv = 1.0 / den
    ps = [e * inv for e in es]
    vws = windows(vbuf)
    ocols = []
    for j in range(DP // LANES):
        acc = None
        for w in range(W):
            t = ps[w] * vws[w][:, j * LANES:(j + 1) * LANES]
            acc = t if acc is None else acc + t
        ocols.append(acc.astype(bf16))
    o = jnp.concatenate(ocols, axis=1)

    kbuf[0:HALO, :] = kbuf[T:T + HALO, :]
    vbuf[0:HALO, :] = vbuf[T:T + HALO, :]

    att = jax.lax.dot_general(woT_s[...], o, NT, preferred_element_type=f32)
    x1 = x + col(2) * att

    m2 = jnp.mean(x1, axis=0, keepdims=True)
    xc2 = x1 - m2
    v2 = jnp.mean(xc2 * xc2, axis=0, keepdims=True)
    h2T = (xc2 * jax.lax.rsqrt(v2 + EPS) * (1.0 + col(4)) + col(3))
    h2 = h2T.T.astype(bf16)

    @pl.when(i == 0)
    def _wait_ffn():
        pltpu.make_async_copy(w1_hbm, w1_s, sems.at[3]).wait()
        pltpu.make_async_copy(w2t_hbm, w2t_s, sems.at[4]).wait()

    acc = None
    for cidx in range(DFF // FC):
        a = jnp.dot(h2, w1_s[:, cidx * FC:(cidx + 1) * FC], preferred_element_type=f32)
        a = jnp.maximum(a, 0.0).astype(bf16)
        t = jax.lax.dot_general(w2t_s[:, cidx * FC:(cidx + 1) * FC], a, NT,
                                preferred_element_type=f32)
        acc = t if acc is None else acc + t
    o_ref[...] = (x1 + col(5) * acc).astype(o_ref.dtype)


@jax.jit
def pallas_adaLN_cond__sliding_local_dilated__dense_activation_relu__prompt_kernel(
    A_x: jax.Array,
    A_wqkv: jax.Array,
    A_wo: jax.Array,
    B_x: jax.Array,
    B_w1: jax.Array,
    B_w2: jax.Array,
    c: jax.Array,
    w_mod: jax.Array,
):
    B, S, D = A_x.shape
    assert B == 1
    DFF = B_w1.shape[1]
    Dh = D // H
    DP = ((Dh + 3) // 4) * 4 * H
    assert DP % LANES == 0
    T = 256
    FC = 768
    xT = jnp.swapaxes(A_x, 1, 2).reshape(D, S)
    w2T = B_w2.T
    f32 = jnp.float32
    bf16 = jnp.bfloat16
    kern = functools.partial(_kernel, T=T, D=D, DP=DP, DFF=DFF, FC=FC)
    any_spec = pl.BlockSpec(memory_space=pltpu.MemorySpace.HBM)
    outT = pl.pallas_call(
        kern,
        grid=(S // T,),
        in_specs=[
            pl.BlockSpec((D, T), lambda i: (0, i)),
            pl.BlockSpec((1, D), lambda i: (0, 0)),
            any_spec, any_spec, any_spec, any_spec, any_spec,
        ],
        out_specs=pl.BlockSpec((D, T), lambda i: (0, i)),
        out_shape=jax.ShapeDtypeStruct((D, S), A_x.dtype),
        scratch_shapes=[
            pltpu.VMEM((D, 3 * D), bf16),
            pltpu.VMEM((D, D), bf16),
            pltpu.VMEM((D, 3 * DP), bf16),
            pltpu.VMEM((D, DP), bf16),
            pltpu.VMEM((D, DFF), bf16),
            pltpu.VMEM((D, DFF), bf16),
            pltpu.VMEM((D, 6 * D), bf16),
            pltpu.VMEM((6 * D, LANES), f32),
            pltpu.VMEM((T + HALO, DP), f32),
            pltpu.VMEM((T + HALO, DP), f32),
            pltpu.SemaphoreType.DMA((5,)),
        ],
        compiler_params=pltpu.CompilerParams(
            dimension_semantics=("arbitrary",),
            vmem_limit_bytes=100 * 1024 * 1024,
        ),
    )(xT, c, A_wqkv, A_wo, B_w1, w2T, w_mod)
    return jnp.swapaxes(outT.reshape(B, D, S), 1, 2)
```
